```python
import os as _os
_os.environ.setdefault("JAX_PLATFORMS", "cpu")
import jax
import jax.numpy as jnp

def _softmax(x, axis=-1):
    return jax.nn.softmax(x, axis=axis)
def _gelu(x):
    return jax.nn.gelu(x, approximate=True)
def _silu(x):
    return jax.nn.silu(x)
def _sigmoid(x):
    return jax.nn.sigmoid(x)
def _layernorm(x, axis=-1, eps=1e-5):
    m = jnp.mean(x, axis=axis, keepdims=True)
    v = jnp.var(x, axis=axis, keepdims=True)
    return (x - m) / jnp.sqrt(v + eps)
def _scatter_add(tgt, idx, src, axis=0):
    return tgt.at[idx].add(src)
def _segment_sum(src, seg, n):
    return jax.ops.segment_sum(src, seg, n)
class _Rng:
    def __init__(self, key):
        self._k = key
    def _next(self):
        self._k, sub = jax.random.split(self._k)
        return sub
    def normal(self, shape):
        return jax.random.normal(self._next(), shape, dtype=jnp.bfloat16)
    def randint(self, lo, hi, shape):
        return jax.random.randint(self._next(), shape, lo, hi, dtype=jnp.int32)
    def uniform(self, shape, lo=0.0, hi=1.0):
        return jax.random.uniform(self._next(), shape, jnp.bfloat16, lo, hi)
    def permutation(self, n):
        return jax.random.permutation(self._next(), n)


kernel_name = 'sequential_preLN__softmax_full_mha__glu_gated_swiglu__prompt'

def setup_inputs():
    _rng = _Rng(jax.random.key(int.from_bytes(__import__("os").urandom(4), "little")))
    _w = (lambda a: (lambda t: t.astype(jnp.bfloat16) if jnp.issubdtype(t.dtype, jnp.floating) else t)(jnp.asarray(a)))
    def _A_setup():
        B, S, D = 1, 2048, 640
        return {
            "x": _w((lambda *s: _rng.normal(s) * 0.05)(B, S, D)),
            "wqkv": _w((lambda *s: _rng.normal(s) * 0.05)(D, 3 * D)),
            "wo": _w((lambda *s: _rng.normal(s) * 0.05)(D, D)),
        }
    _A_in = _A_setup()

    def _B_setup():
        B, S, D, F = 1, 2048, 640, 1728
        return {
            "x": _w((lambda *s: _rng.normal(s) * 0.05)(B, S, D)),
            "w1": _w((lambda *s: _rng.normal(s) * 0.05)(D, F) * (2.0 / D) ** 0.5),
            "w3": _w((lambda *s: _rng.normal(s) * 0.05)(D, F) * (2.0 / D) ** 0.5),
            "w2": _w((lambda *s: _rng.normal(s) * 0.05)(F, D) * (2.0 / F) ** 0.5),
        }
    _B_in = _B_setup()

    return {
        "A_x": _A_in["x"],
        "A_wqkv": _A_in["wqkv"],
        "A_wo": _A_in["wo"],
        "B_x": _B_in["x"],
        "B_w1": _B_in["w1"],
        "B_w3": _B_in["w3"],
        "B_w2": _B_in["w2"],
    }

def reference(A_x, A_wqkv, A_wo, B_x, B_w1, B_w3, B_w2):
    def _A_ref(x, wqkv, wo):
        B, S, D = x.shape
        H = 32; Dh = D // H
        qkv = (lambda x, *d: x.transpose(*d))((x @ wqkv).reshape(B, S, 3, H, Dh), 2, 0, 3, 1, 4)
        q, k, v = qkv[0], qkv[1], qkv[2]
        scale = Dh ** -0.5
        scores = jnp.einsum("bhqd,bhkd->bhqk", q, k) * scale
        p = _softmax(scores, axis=-1)
        o = jnp.einsum("bhqk,bhkd->bhqd", p, v)
        return (lambda x, *d: x.transpose(*d))(o, 0, 2, 1, 3).reshape(B, S, D) @ wo

    def _B_ref(x, w1, w3, w2):
        gate = jnp.einsum("bsd,df->bsf", x, w1)
        up = jnp.einsum("bsd,df->bsf", x, w3)
        h = _silu(gate) * up
        out = jnp.einsum("bsf,fd->bsd", h, w2)
        return out

    x = A_x
    h = x + _A_ref(_layernorm(x, axis=-1), A_wqkv, A_wo)
    h2 = h + _B_ref(_layernorm(h, axis=-1), B_w1, B_w3, B_w2)
    return h2
```

```python
import functools

import jax
import jax.numpy as jnp
import numpy as np
from jax import lax
from jax.experimental import pallas as pl
from jax.experimental.pallas import tpu as pltpu

S = 2048
D = 640
H = 32
DH = D // H
F = 1728
FM = 1664
BQ = 512
NQ = S // BQ
KC = 128
NKT = S // KC
RB = 512
NRB = S // RB
EPS = 1e-5
QSCALE = float(DH ** -0.5 * np.log2(np.e))
NT = (((1,), (1,)), ((), ()))
NN = (((1,), (0,)), ((), ()))
VTILES = tuple(range(6, 16))
LAG = 16
LNC = 128
UNROLL_A = True
UNROLL_C = True
SCOPES = False

bf16 = jnp.bfloat16
f32 = jnp.float32
i32 = jnp.int32


class _noscope:
    def __enter__(self):
        return None

    def __exit__(self, *a):
        return False


def scope(name):
    return jax.named_scope(name) if SCOPES else _noscope()


def _layernorm(x):
    mu = jnp.mean(x, axis=-1, keepdims=True)
    xc = x - mu
    var = jnp.mean(xc * xc, axis=-1, keepdims=True)
    return xc * lax.rsqrt(var + EPS)


def _kernel(x_hbm, wqkv_hbm, wo_hbm, w1_hbm, w3_hbm, w2_hbm, out_hbm,
            x_v, xn_v, h_v, wqkv_v, wqvt_v, wo_v, w13_v, w2_v,
            ks, qt32, qtp, vt, ot, p0, p1, sbuf, ob, lbuf, vflag, sems, osems):
    def x_copy(r):
        rows = pl.ds(r * RB, RB)
        return pltpu.make_async_copy(x_hbm.at[rows, :], x_v.at[rows, :], sems.at[r])

    def w_copy(t):
        cols = pl.ds(t * D, D)
        return pltpu.make_async_copy(wqkv_hbm.at[:, cols], wqkv_v.at[:, cols], sems.at[4 + t])

    wo_cp = pltpu.make_async_copy(wo_hbm, wo_v, sems.at[7])
    w13_cps = [
        pltpu.make_async_copy(w1_hbm.at[pl.ds(0, FM), :], w13_v.at[pl.ds(0, FM), :], sems.at[8]),
        pltpu.make_async_copy(w3_hbm.at[pl.ds(0, FM), :], w13_v.at[pl.ds(FM, FM), :], sems.at[9]),
        pltpu.make_async_copy(w1_hbm.at[pl.ds(FM, F - FM), :], w13_v.at[pl.ds(2 * FM, F - FM), :], sems.at[10]),
        pltpu.make_async_copy(w3_hbm.at[pl.ds(FM, F - FM), :], w13_v.at[pl.ds(2 * FM + F - FM, F - FM), :], sems.at[11]),
    ]
    w2_cp = pltpu.make_async_copy(w2_hbm, w2_v, sems.at[12])
    x_copy(0).start()
    w_copy(1).start()

    lane = lax.broadcasted_iota(i32, (1, 128), 1)

    def rows_of(r):
        return slice(r * RB, (r + 1) * RB)

    def ln1(r0, r1):
        for c0 in range(r0, r1, LNC):
            rows = slice(c0, c0 + LNC)
            xn_v[rows, :] = _layernorm(x_v[rows, :].astype(f32)).astype(bf16)

    def k_proj(r0, r1):
        prow = slice(r0 // 2, r1 // 2)
        k = jnp.dot(xn_v[r0:r1, :], wqkv_v[:, D:2 * D], preferred_element_type=f32)
        kp = pltpu.bitcast(k.astype(bf16), i32)
        parts = [kp[:, j * 128:(j + 1) * 128] for j in range(5)]
        for j in range(5):
            ks[j, prow, :] = parts[j]
        for j in range(4):
            ks[5 + j, prow, :] = jnp.where(lane >= 64, parts[j], parts[j + 1])

    def qv_proj(r0, r1):
        rows = slice(r0, r1)
        qv = lax.dot_general(wqvt_v[...], xn_v[rows, :], NT, preferred_element_type=f32)
        q = qv[0:D, :] * QSCALE
        qt32[:, rows] = q
        qtp[:, rows] = pltpu.bitcast(q.astype(bf16), i32)
        v = qv[D:2 * D, :].astype(bf16).astype(f32)
        vt[:, rows] = v
        vbits = pltpu.bitcast(v, i32) & 0x7FFFFFFF
        vmax = jnp.max(vbits.reshape(D // 8, 8, r1 - r0), axis=0)
        vflag[:, rows] = vmax

    with scope("phaseA"):
        x_copy(0).wait()
        ln1(0, 512)
        w_copy(1).wait()
        x_copy(1).start()
        k_proj(0, 256)
        x_copy(1).wait()
        x_copy(2).start()
        x_copy(3).start()
        k_proj(256, 384)
        ln1(512, 1024)
        k_proj(512, 960)
        x_copy(2).wait()
        x_copy(3).wait()
        w_copy(0).start()
        w_copy(2).start()
        k_proj(384, 512)
        ln1(1024, 2048)
        k_proj(1024, 1536)
        k_proj(1536, 2048)
        w_copy(0).wait()
        w_copy(2).wait()
        wo_cp.start()
        for cp in w13_cps:
            cp.start()
        w2_cp.start()
        k_proj(960, 1024)
        wqvt_v[0:D, :] = wqkv_v[:, 0:D].astype(f32).T.astype(bf16)
        wqvt_v[D:2 * D, :] = wqkv_v[:, 2 * D:3 * D].astype(f32).T.astype(bf16)
        for r in range(NRB):
            qv_proj(r * RB, (r + 1) * RB)

    row24 = lax.broadcasted_iota(i32, (24, 1), 0)
    prow64 = lax.broadcasted_iota(i32, (64, 1), 0)

    def head_params(h):
        c0 = h * DH
        j = c0 >> 7
        o = c0 & 127
        straddle = o > 128 - DH
        slab = jnp.where(straddle, 5 + j, j)
        lo_base = jnp.where(straddle, j + 1, j) * 64
        hi_base = j * 64 + 32
        return slab, o, lo_base, hi_base

    def qcols(qb):
        if isinstance(qb, int):
            return slice(qb * BQ, (qb + 1) * BQ)
        return pl.ds(pl.multiple_of(qb * BQ, BQ), BQ)

    def load_q(h, qb):
        slab, o, lo_base, hi_base = head_params(h)
        lo = qtp[pl.ds(pl.multiple_of(lo_base, 32), 32), qcols(qb)]
        hi = qtp[pl.ds(pl.multiple_of(hi_base, 32), 32), qcols(qb)]
        q = jnp.concatenate([lo, hi], axis=0)
        m = ((2 * prow64 - o) & 127) < DH
        return pltpu.bitcast(jnp.where(m, q, 0), bf16), slab

    def k_bcast(h):
        slab, o, _, _ = head_params(h)
        out = {}
        for c in VTILES:
            kk = ks[slab, (c * KC + KC - 16) // 2:(c * KC + KC) // 2, :]
            kk = pltpu.roll(kk, (128 - o) & 127, 1)
            x = pltpu.bitcast(kk, bf16).astype(f32)
            out[c] = [jnp.broadcast_to(x[:, d:d + 1], (16, 128)) for d in range(DH)]
        return out

    def q_bcast(h, qb):
        return [jnp.broadcast_to(qt32[pl.ds(h * DH + d, 1), qcols(qb)], (8, BQ)) for d in range(DH)]

    def vt_params(h):
        c0 = h * DH
        r0 = c0 & ~7
        o = c0 - r0
        rsum = jnp.where(o == 0, DH, 0)
        return r0, o, rsum

    def vt_tile(r0, rsum, c):
        v = vt[pl.ds(pl.multiple_of(r0, 8), 24), c * KC:(c + 1) * KC]
        return jnp.where(row24 == rsum, 1.0, v)

    def finish(acc, h, qb, check):
        r0, o, rsum = vt_params(h)
        l = jnp.sum(jnp.where(row24 == rsum, acc, 0.0), axis=0, keepdims=True)
        res = acc * (1.0 / l)
        first = pl.ds(pl.multiple_of(r0, 8), 8)
        old = ot[first, qcols(qb)]
        ot[first, qcols(qb)] = jnp.where(row24[0:8] < o, old, res[0:8])
        ot[pl.ds(pl.multiple_of(r0 + 8, 8), 16), qcols(qb)] = res[8:24]
        if check:
            lbuf[pl.ds(h * NQ + qb, 1), :] = l

    def step(a_item, p_a, c_item, p_c, kb, chain):
        if a_item is not None:
            q, slab = load_q(*a_item)
        if c_item is not None:
            r0, _, rsum = vt_params(c_item[0])
            qb_ = q_bcast(*c_item)
            acc = None
            prev = chain[0]
        for c in range(NKT):
            mr = KC - 16 if c in VTILES else KC
            prows = slice(c * KC // 2, (c * KC + mr) // 2)
            if c_item is not None:
                pp = pltpu.bitcast(p_c[prows, :], bf16)
                if c in VTILES:
                    outs = []
                    for j in range(BQ // 128):
                        accs = [None if prev is None else prev[r] * 0.0 for r in range(2)]
                        for d in range(DH):
                            qv = qb_[d][:, j * 128:(j + 1) * 128]
                            for r in range(2):
                                t = kb[c][d][r * 8:(r + 1) * 8, :] * qv
                                accs[r] = t if accs[r] is None else accs[r] + t
                            if d == LAG - 1:
                                prev = list(accs)
                        outs.append(jnp.concatenate(accs, axis=0))
                    sv = jnp.concatenate(outs, axis=1)
                    pp = jnp.concatenate([pp, jnp.exp2(sv).astype(bf16)], axis=0)
                d_ = lax.dot_general(vt_tile(r0, rsum, c), pp, NN, preferred_element_type=f32)
                acc = d_ if acc is None else acc + d_
            if a_item is not None:
                kk = pltpu.bitcast(ks[slab, prows, :], bf16)
                s = jnp.dot(kk, q, preferred_element_type=f32)
                p_a[prows, :] = pltpu.bitcast(jnp.exp2(s).astype(bf16), i32)
        if c_item is not None:
            finish(acc, *c_item, check=True)
            chain[0] = prev

    with scope("attpro"):
        step((0, 0), p0, None, None, None, None)

    def att_body(h, carry):
        kb = k_bcast(h)
        ch = [None]
        step((h, 1), p1, (h, 0), p0, kb, ch)
        step((h, 2), p0, (h, 1), p1, kb, ch)
        step((h, 3), p1, (h, 2), p0, kb, ch)
        step((h + 1, 0), p0, (h, 3), p1, kb, ch)
        return carry

    with scope("attloop"):
        lax.fori_loop(0, H - 1, att_body, 0)
    with scope("attepi"):
        hl = H - 1
        kb = k_bcast(hl)
        ch = [None]
        step((hl, 1), p1, (hl, 0), p0, kb, ch)
        step((hl, 2), p0, (hl, 1), p1, kb, ch)
        step((hl, 3), p1, (hl, 2), p0, kb, ch)
        step(None, None, (hl, 3), p1, kb, ch)

    lv = lbuf[...]
    l_ok = jnp.min(jnp.where((lv >= 2.0 ** -60) & (lv <= 2.0 ** 60), 1.0, 0.0))
    v_ok = jnp.where(jnp.max(vflag[...]) <= 0x5D800000, 1.0, 0.0)

    @pl.when(jnp.minimum(l_ok, v_ok) < 0.5)
    def _():
        def slow(i, c):
            h = i >> 2
            qb = i & 3
            q, slab = load_q(h, qb)
            s = jnp.dot(pltpu.bitcast(ks[slab], bf16), q, preferred_element_type=f32)
            sbuf[...] = s
            m = jnp.max(sbuf[...], axis=0, keepdims=True)
            p0[...] = pltpu.bitcast(jnp.exp2(sbuf[...] - m).astype(bf16), i32)
            r0, _, rsum = vt_params(h)
            v = vt[pl.ds(pl.multiple_of(r0, 8), 24), :]
            v = jnp.where(row24 == rsum, 1.0, v)
            acc = lax.dot_general(v, pltpu.bitcast(p0[...], bf16), NN, preferred_element_type=f32)
            finish(acc, h, qb, check=False)
            return c
        lax.fori_loop(0, H * NQ, slow, 0)

    wo_cp.wait()
    for cp in w13_cps:
        cp.wait()
    w2_cp.wait()

    def out_copy(r):
        rows = pl.ds(r * RB, RB) if isinstance(r, int) else pl.ds(pl.multiple_of(r * RB, RB), RB)
        return pltpu.make_async_copy(ob.at[rows, :], out_hbm.at[rows, :], osems.at[r])

    def stage1(r):
        rows = rows_of(r)
        o = ot[:, rows].T.astype(bf16)
        h = x_v[rows, :].astype(f32) + jnp.dot(o, wo_v[...], preferred_element_type=f32)
        h_v[rows, :] = h
        xn_v[rows, :] = _layernorm(h).astype(bf16)

    def stage2(r):
        rows = rows_of(r)
        gu = lax.dot_general(xn_v[rows, :], w13_v[...], NT, preferred_element_type=f32)
        g = gu[:, 0:FM]
        u = gu[:, FM:2 * FM]
        t = gu[:, 2 * FM:2 * F]
        hh_main = (g * jax.nn.sigmoid(g) * u).astype(bf16)
        tg = t[:, 0:F - FM]
        tu = t[:, F - FM:2 * (F - FM)]
        hh_last = (tg * jax.nn.sigmoid(tg) * tu).astype(bf16)
        hh = jnp.concatenate([hh_main, hh_last], axis=1)
        out = h_v[rows, :] + jnp.dot(hh, w2_v[...], preferred_element_type=f32)
        ob[rows, :] = out.astype(bf16)
        out_copy(r).start()

    with scope("phaseC"):
        stage1(0)
        for r in range(NRB):
            if r + 1 < NRB:
                stage1(r + 1)
            stage2(r)
    with scope("outwait"):
        for r in range(NRB):
            out_copy(r).wait()


@jax.jit
def pallas_sequential_preLN__softmax_full_mha__glu_gated_swiglu__prompt_kernel(
    A_x: jax.Array,
    A_wqkv: jax.Array,
    A_wo: jax.Array,
    B_x: jax.Array,
    B_w1: jax.Array,
    B_w3: jax.Array,
    B_w2: jax.Array,
):
    del B_x
    x = A_x.reshape(S, D)
    hbm = pl.BlockSpec(memory_space=pltpu.HBM)
    out = pl.pallas_call(
        _kernel,
        out_shape=jax.ShapeDtypeStruct((S, D), bf16),
        in_specs=[hbm] * 6,
        out_specs=hbm,
        scratch_shapes=[
            pltpu.VMEM((S, D), bf16),
            pltpu.VMEM((S, D), bf16),
            pltpu.VMEM((S, D), f32),
            pltpu.VMEM((D, 3 * D), bf16),
            pltpu.VMEM((2 * D, D), bf16),
            pltpu.VMEM((D, D), bf16),
            pltpu.VMEM((2 * F, D), bf16),
            pltpu.VMEM((F, D), bf16),
            pltpu.VMEM((9, S // 2, 128), i32),
            pltpu.VMEM((D, S), f32),
            pltpu.VMEM((D // 2, S), i32),
            pltpu.VMEM((D, S), f32),
            pltpu.VMEM((D, S), f32),
            pltpu.VMEM((S // 2, BQ), i32),
            pltpu.VMEM((S // 2, BQ), i32),
            pltpu.VMEM((S, BQ), f32),
            pltpu.VMEM((S, D), bf16),
            pltpu.VMEM((H * NQ, BQ), f32),
            pltpu.VMEM((8, S), i32),
            pltpu.SemaphoreType.DMA((13,)),
            pltpu.SemaphoreType.DMA((NRB,)),
        ],
        compiler_params=pltpu.CompilerParams(vmem_limit_bytes=120 * 1024 * 1024),
        name="fused_block",
    )(x, A_wqkv, A_wo, B_w1.T, B_w3.T, B_w2)
    return out.reshape(1, S, D)
```

```python
import jax
import jax.numpy as jnp
import numpy as np
from jax import lax
from jax.experimental import pallas as pl
from jax.experimental.pallas import tpu as pltpu

S = 2048
D = 640
H = 32
DH = D // H
F = 1728
FM = 1664
BQ = 512
NQ = S // BQ
KC = 128
NKT = S // KC
RB = 512
NRB = S // RB
EPS = 1e-5
QSCALE = float(DH ** -0.5 * np.log2(np.e))
NT = (((1,), (1,)), ((), ()))
NN = (((1,), (0,)), ((), ()))
VTILES = tuple(range(6, 16))
LAG = 16
HPB = 3
LNC = 128
LASTP = 4
KGROUPS = ((0, 1), (1, 3), (3, 5))
KP = 128

bf16 = jnp.bfloat16
f32 = jnp.float32
i32 = jnp.int32


def _layernorm(x):
    mu = jnp.mean(x, axis=-1, keepdims=True)
    xc = x - mu
    var = jnp.mean(xc * xc, axis=-1, keepdims=True)
    return xc * lax.rsqrt(var + EPS)


def _kernel(x_hbm, wqkv_hbm, wo_hbm, w1_hbm, w3_hbm, w2_hbm, out_hbm,
            x_v, xn_v, h_v, wqkv_v, wqvt_v, wo_v, w13_v, w2_v,
            ks, qt32, qtp, vt, ot, p0, p1, sbuf, ob, lbuf, vflag, sems, osems):
    def x_copy(r):
        rows = pl.ds(r * RB, RB)
        return pltpu.make_async_copy(x_hbm.at[rows, :], x_v.at[rows, :], sems.at[r])

    def w_copy(t):
        cols = pl.ds(t * D, D)
        return pltpu.make_async_copy(wqkv_hbm.at[:, cols], wqkv_v.at[:, cols], sems.at[4 + t])

    def wk_copy(n):
        cols = pl.ds(D + n * 128, 128)
        return pltpu.make_async_copy(wqkv_hbm.at[:, cols], wqkv_v.at[:, cols], sems.at[13 + n])

    wo_cp = pltpu.make_async_copy(wo_hbm, wo_v, sems.at[7])
    w13_cps = [
        pltpu.make_async_copy(w1_hbm.at[pl.ds(0, FM), :], w13_v.at[pl.ds(0, FM), :], sems.at[8]),
        pltpu.make_async_copy(w3_hbm.at[pl.ds(0, FM), :], w13_v.at[pl.ds(FM, FM), :], sems.at[9]),
        pltpu.make_async_copy(w1_hbm.at[pl.ds(FM, F - FM), :], w13_v.at[pl.ds(2 * FM, F - FM), :], sems.at[10]),
        pltpu.make_async_copy(w3_hbm.at[pl.ds(FM, F - FM), :], w13_v.at[pl.ds(FM + F, F - FM), :], sems.at[11]),
    ]
    w2_cp = pltpu.make_async_copy(w2_hbm, w2_v, sems.at[12])
    x_copy(0).start()
    for n in range(5):
        wk_copy(n).start()

    lane = lax.broadcasted_iota(i32, (1, 128), 1)

    def rows_of(r):
        return slice(r * RB, (r + 1) * RB)

    def ln1(r0, r1):
        for c0 in range(r0, r1, LNC):
            rows = slice(c0, c0 + LNC)
            xn_v[rows, :] = _layernorm(x_v[rows, :].astype(f32)).astype(bf16)

    def k_proj(r0, r1):
        prow = slice(r0 // 2, r1 // 2)
        k = jnp.dot(xn_v[r0:r1, :], wqkv_v[:, D:2 * D], preferred_element_type=f32)
        kp = pltpu.bitcast(k.astype(bf16), i32)
        parts = [kp[:, j * 128:(j + 1) * 128] for j in range(5)]
        for j in range(5):
            ks[j, prow, :] = parts[j]
        for j in range(4):
            ks[5 + j, prow, :] = jnp.where(lane >= 64, parts[j], parts[j + 1])

    def qv_proj(r0, r1):
        rows = slice(r0, r1)
        qv = lax.dot_general(wqvt_v[...], xn_v[rows, :], NT, preferred_element_type=f32)
        q = qv[0:D, :] * QSCALE
        qt32[:, rows] = q
        qtp[:, rows] = pltpu.bitcast(q.astype(bf16), i32)
        v = qv[D:2 * D, :].astype(bf16).astype(f32)
        vt[:, rows] = v
        vbits = pltpu.bitcast(v, i32) & 0x7FFFFFFF
        vflag[:, rows] = jnp.max(vbits.reshape(D // 8, 8, r1 - r0), axis=0)

    x_copy(0).wait()
    ln1(0, 512)
    first = []
    for gi, (n0, n1) in enumerate(KGROUPS):
        for n in range(n0, n1):
            wk_copy(n).wait()
        if gi == 1:
            x_copy(1).start()
        kn = jnp.dot(xn_v[0:256, :], wqkv_v[:, D + n0 * 128:D + n1 * 128], preferred_element_type=f32)
        knp = pltpu.bitcast(kn.astype(bf16), i32)
        for n in range(n0, n1):
            first.append(knp[:, (n - n0) * 128:(n - n0 + 1) * 128])
            ks[n, 0:128, :] = first[n]
    for j in range(4):
        ks[5 + j, 0:128, :] = jnp.where(lane >= 64, first[j], first[j + 1])
    x_copy(1).wait()
    x_copy(2).start()
    x_copy(3).start()
    k_proj(256, 512)
    ln1(512, 1024)
    for c0 in range(512, 1024, KP):
        k_proj(c0, c0 + KP)
    x_copy(2).wait()
    x_copy(3).wait()
    w_copy(0).start()
    w_copy(2).start()
    ln1(1024, 2048)
    for c0 in range(1024, 1920, KP):
        k_proj(c0, min(c0 + KP, 1920))
    w_copy(0).wait()
    w_copy(2).wait()
    wo_cp.start()
    for cp in w13_cps:
        cp.start()
    w2_cp.start()
    k_proj(1920, 2048)
    wqvt_v[0:D, :] = wqkv_v[:, 0:D].astype(f32).T.astype(bf16)
    wqvt_v[D:2 * D, :] = wqkv_v[:, 2 * D:3 * D].astype(f32).T.astype(bf16)
    for r in range(NRB):
        qv_proj(r * RB, (r + 1) * RB)

    row24 = lax.broadcasted_iota(i32, (24, 1), 0)
    prow64 = lax.broadcasted_iota(i32, (64, 1), 0)

    def head_params(h):
        c0 = h * DH
        j = c0 >> 7
        o = c0 & 127
        straddle = o > 128 - DH
        slab = jnp.where(straddle, 5 + j, j)
        lo_base = jnp.where(straddle, j + 1, j) * 64
        hi_base = j * 64 + 32
        return slab, o, lo_base, hi_base

    def qcols(qb):
        if isinstance(qb, int):
            return slice(qb * BQ, (qb + 1) * BQ)
        return pl.ds(pl.multiple_of(qb * BQ, BQ), BQ)

    def load_q(h, qb):
        slab, o, lo_base, hi_base = head_params(h)
        lo = qtp[pl.ds(pl.multiple_of(lo_base, 32), 32), qcols(qb)]
        hi = qtp[pl.ds(pl.multiple_of(hi_base, 32), 32), qcols(qb)]
        q = jnp.concatenate([lo, hi], axis=0)
        m = ((2 * prow64 - o) & 127) < DH
        return pltpu.bitcast(jnp.where(m, q, 0), bf16), slab

    def k_bcast(h):
        slab, o, _, _ = head_params(h)
        out = {}
        for c in VTILES:
            kk = ks[slab, (c * KC + KC - 16) // 2:(c * KC + KC) // 2, :]
            kk = pltpu.roll(kk, (128 - o) & 127, 1)
            x = pltpu.bitcast(kk, bf16).astype(f32)
            out[c] = [jnp.broadcast_to(x[:, d:d + 1], (16, 128)) for d in range(DH)]
        return out

    def q_bcast(h, qb):
        return [jnp.broadcast_to(qt32[pl.ds(h * DH + d, 1), qcols(qb)], (8, BQ)) for d in range(DH)]

    def vt_params(h):
        c0 = h * DH
        r0 = c0 & ~7
        o = c0 - r0
        rsum = jnp.where(o == 0, DH, 0)
        return r0, o, rsum

    def vt_tile(r0, rsum, c):
        v = vt[pl.ds(pl.multiple_of(r0, 8), 24), c * KC:(c + 1) * KC]
        return jnp.where(row24 == rsum, 1.0, v)

    def finish(acc, h, qb, check):
        r0, o, rsum = vt_params(h)
        l = jnp.sum(jnp.where(row24 == rsum, acc, 0.0), axis=0, keepdims=True)
        res = acc * (1.0 / l)
        first_rows = pl.ds(pl.multiple_of(r0, 8), 8)
        old = ot[first_rows, qcols(qb)]
        ot[first_rows, qcols(qb)] = jnp.where(row24[0:8] < o, old, res[0:8])
        ot[pl.ds(pl.multiple_of(r0 + 8, 8), 16), qcols(qb)] = res[8:24]
        if check:
            lbuf[pl.ds(h * NQ + qb, 1), :] = l

    def step(a_item, p_a, c_item, p_c, kb, chain, va=VTILES, vc=VTILES):
        if a_item is not None:
            q, slab = load_q(*a_item)
        if c_item is not None:
            r0, _, rsum = vt_params(c_item[0])
            qb_ = q_bcast(*c_item) if vc else None
            acc = None
            prev = chain[0]
        for c in range(NKT):
            if c_item is not None:
                mr = KC - 16 if c in vc else KC
                pp = pltpu.bitcast(p_c[c * KC // 2:(c * KC + mr) // 2, :], bf16)
                if c in vc:
                    outs = []
                    for j in range(BQ // 128):
                        accs = [None if prev is None else prev[r] * 0.0 for r in range(2)]
                        for d in range(DH):
                            qv = qb_[d][:, j * 128:(j + 1) * 128]
                            for r in range(2):
                                t = kb[c][d][r * 8:(r + 1) * 8, :] * qv
                                accs[r] = t if accs[r] is None else accs[r] + t
                            if d == LAG - 1:
                                prev = list(accs)
                        outs.append(jnp.concatenate(accs, axis=0))
                    sv = jnp.concatenate(outs, axis=1)
                    pp = jnp.concatenate([pp, jnp.exp2(sv).astype(bf16)], axis=0)
                d_ = lax.dot_general(vt_tile(r0, rsum, c), pp, NN, preferred_element_type=f32)
                acc = d_ if acc is None else acc + d_
            if a_item is not None:
                mr = KC - 16 if c in va else KC
                prows = slice(c * KC // 2, (c * KC + mr) // 2)
                kk = pltpu.bitcast(ks[slab, prows, :], bf16)
                s = jnp.dot(kk, q, preferred_element_type=f32)
                p_a[prows, :] = pltpu.bitcast(jnp.exp2(s).astype(bf16), i32)
        if c_item is not None:
            finish(acc, *c_item, check=True)
            chain[0] = prev

    def head_steps(h, ch):
        kb = k_bcast(h)
        step((h, 1), p1, (h, 0), p0, kb, ch)
        step((h, 2), p0, (h, 1), p1, kb, ch)
        step((h, 3), p1, (h, 2), p0, kb, ch)
        step((h + 1, 0), p0, (h, 3), p1, kb, ch)

    def att_body(t, carry):
        ch = [None]
        for i in range(HPB):
            head_steps(t * HPB + i, ch)
        return carry

    step((0, 0), p0, None, None, None, None)
    lax.fori_loop(0, (H - 1) // HPB, att_body, 0)
    for h in range((H - 1) // HPB * HPB, H - 1):
        head_steps(h, [None])
    hl = H - 1
    kb = k_bcast(hl)
    ch = [None]
    step((hl, 1), p1, (hl, 0), p0, kb, ch)
    step((hl, 2), p0, (hl, 1), p1, kb, ch)
    step((hl, 3), p1, (hl, 2), p0, kb, ch, va=())
    step(None, None, (hl, 3), p1, kb, ch, vc=())

    lv = lbuf[...]
    l_ok = jnp.min(jnp.where((lv >= 2.0 ** -80) & (lv <= 2.0 ** 80), 1.0, 0.0))
    v_ok = jnp.where(jnp.max(vflag[...]) <= 0x53800000, 1.0, 0.0)

    @pl.when(jnp.minimum(l_ok, v_ok) < 0.5)
    def _():
        def slow(i, c):
            h = i >> 2
            qb = i & 3
            q, slab = load_q(h, qb)
            sbuf[...] = jnp.dot(pltpu.bitcast(ks[slab], bf16), q, preferred_element_type=f32)
            m = jnp.max(sbuf[...], axis=0, keepdims=True)
            p0[...] = pltpu.bitcast(jnp.exp2(sbuf[...] - m).astype(bf16), i32)
            r0, _, rsum = vt_params(h)
            v = vt[pl.ds(pl.multiple_of(r0, 8), 24), :]
            v = jnp.where(row24 == rsum, 1.0, v)
            acc = lax.dot_general(v, pltpu.bitcast(p0[...], bf16), NN, preferred_element_type=f32)
            finish(acc, h, qb, check=False)
            return c
        lax.fori_loop(0, H * NQ, slow, 0)

    wo_cp.wait()
    for cp in w13_cps:
        cp.wait()
    w2_cp.wait()

    def out_copy(r0, n, sem):
        return pltpu.make_async_copy(ob.at[pl.ds(r0, n), :], out_hbm.at[pl.ds(r0, n), :], osems.at[sem])

    def stage1(r):
        rows = rows_of(r)
        o = ot[:, rows].T.astype(bf16)
        h = x_v[rows, :].astype(f32) + jnp.dot(o, wo_v[...], preferred_element_type=f32)
        h_v[rows, :] = h
        xn_v[rows, :] = _layernorm(h).astype(bf16)

    def stage2(r):
        rows = rows_of(r)
        gu = lax.dot_general(xn_v[rows, :], w13_v[...], NT, preferred_element_type=f32)
        g = gu[:, 0:FM]
        u = gu[:, FM:2 * FM]
        t = gu[:, 2 * FM:2 * F]
        hh_main = (g * jax.nn.sigmoid(g) * u).astype(bf16)
        tg = t[:, 0:F - FM]
        tu = t[:, F - FM:2 * (F - FM)]
        hh_last = (tg * jax.nn.sigmoid(tg) * tu).astype(bf16)
        hh = jnp.concatenate([hh_main, hh_last], axis=1)
        pieces = LASTP if r == NRB - 1 else 1
        pr = RB // pieces
        for i in range(pieces):
            sub = slice(r * RB + i * pr, r * RB + (i + 1) * pr)
            out = h_v[sub, :] + jnp.dot(hh[i * pr:(i + 1) * pr, :], w2_v[...], preferred_element_type=f32)
            ob[sub, :] = out.astype(bf16)
            out_copy(r * RB + i * pr, pr, r + i).start()

    stage1(0)
    for r in range(NRB):
        if r + 1 < NRB:
            stage1(r + 1)
        stage2(r)
    for r in range(NRB - 1):
        out_copy(r * RB, RB, r).wait()
    for i in range(LASTP):
        out_copy((NRB - 1) * RB + i * (RB // LASTP), RB // LASTP, NRB - 1 + i).wait()


@jax.jit
def pallas_sequential_preLN__softmax_full_mha__glu_gated_swiglu__prompt_kernel(
    A_x: jax.Array,
    A_wqkv: jax.Array,
    A_wo: jax.Array,
    B_x: jax.Array,
    B_w1: jax.Array,
    B_w3: jax.Array,
    B_w2: jax.Array,
):
    del B_x
    hbm = pl.BlockSpec(memory_space=pltpu.HBM)
    out = pl.pallas_call(
        _kernel,
        out_shape=jax.ShapeDtypeStruct((S, D), bf16),
        in_specs=[hbm] * 6,
        out_specs=hbm,
        scratch_shapes=[
            pltpu.VMEM((S, D), bf16),
            pltpu.VMEM((S, D), bf16),
            pltpu.VMEM((S, D), f32),
            pltpu.VMEM((D, 3 * D), bf16),
            pltpu.VMEM((2 * D, D), bf16),
            pltpu.VMEM((D, D), bf16),
            pltpu.VMEM((2 * F, D), bf16),
            pltpu.VMEM((F, D), bf16),
            pltpu.VMEM((9, S // 2, 128), i32),
            pltpu.VMEM((D, S), f32),
            pltpu.VMEM((D // 2, S), i32),
            pltpu.VMEM((D, S), f32),
            pltpu.VMEM((D, S), f32),
            pltpu.VMEM((S // 2, BQ), i32),
            pltpu.VMEM((S // 2, BQ), i32),
            pltpu.VMEM((S, BQ), f32),
            pltpu.VMEM((S, D), bf16),
            pltpu.VMEM((H * NQ, BQ), f32),
            pltpu.VMEM((8, S), i32),
            pltpu.SemaphoreType.DMA((18,)),
            pltpu.SemaphoreType.DMA((NRB - 1 + LASTP,)),
        ],
        compiler_params=pltpu.CompilerParams(vmem_limit_bytes=120 * 1024 * 1024),
        name="fused_block",
    )(A_x.reshape(S, D), A_wqkv, A_wo, B_w1.T, B_w3.T, B_w2)
    return out.reshape(1, S, D)
```
